```python
import os as _os
_os.environ.setdefault("JAX_PLATFORMS", "cpu")
import jax
import jax.numpy as jnp

def _softmax(x, axis=-1):
    return jax.nn.softmax(x, axis=axis)
def _gelu(x):
    return jax.nn.gelu(x, approximate=True)
def _silu(x):
    return jax.nn.silu(x)
def _sigmoid(x):
    return jax.nn.sigmoid(x)
def _layernorm(x, axis=-1, eps=1e-5):
    m = jnp.mean(x, axis=axis, keepdims=True)
    v = jnp.var(x, axis=axis, keepdims=True)
    return (x - m) / jnp.sqrt(v + eps)
def _scatter_add(tgt, idx, src, axis=0):
    return tgt.at[idx].add(src)
def _segment_sum(src, seg, n):
    return jax.ops.segment_sum(src, seg, n)
class _Rng:
    def __init__(self, key):
        self._k = key
    def _next(self):
        self._k, sub = jax.random.split(self._k)
        return sub
    def normal(self, shape):
        return jax.random.normal(self._next(), shape, dtype=jnp.bfloat16)
    def randint(self, lo, hi, shape):
        return jax.random.randint(self._next(), shape, lo, hi, dtype=jnp.int32)
    def uniform(self, shape, lo=0.0, hi=1.0):
        return jax.random.uniform(self._next(), shape, jnp.bfloat16, lo, hi)
    def permutation(self, n):
        return jax.random.permutation(self._next(), n)


kernel_name = 'standalone__gqa_block_cached__sampling'

def setup_inputs():
    _rng = _Rng(jax.random.key(int.from_bytes(__import__("os").urandom(4), "little")))
    _w = (lambda a: (lambda t: t.astype(jnp.bfloat16) if jnp.issubdtype(t.dtype, jnp.floating) else t)(jnp.asarray(a)))
    B, Sq, D = 32, 16, 1024
    Hq, Hkv, Sk, Dh = 32, 4, 2048, 128
    assert Hq % Hkv == 0, (Hq, Hkv)
    return {
        "x": _w((lambda *s: _rng.normal(s) * 0.8)(B, Sq, D)),
        "k_cache": _w((lambda *s: _rng.normal(s) * 0.8)(B, Hkv, Sk, Dh)),
        "v_cache": _w((lambda *s: _rng.normal(s) * 0.05)(B, Hkv, Sk, Dh)),
        "wq": _w((lambda *s: _rng.normal(s) * 0.8)(D, Hq * Dh) * (D ** -0.5)),
        "wo": _w((lambda *s: _rng.normal(s) * 0.05)(Hq * Dh, D) * ((Hq * Dh) ** -0.5)),
    }

def reference(x, k_cache, v_cache, wq, wo):
    B, Sq, D = x.shape
    Hq, Dh = 32, 128
    Hkv = k_cache.shape[1]
    rep = Hq // Hkv
    q = (lambda x, *d: x.transpose(*d))((x @ wq).reshape(B, Sq, Hq, Dh), 0, 2, 1, 3)
    k = jnp.repeat(k_cache, rep, axis=1)
    v = jnp.repeat(v_cache, rep, axis=1)
    scores = jnp.einsum("bhqd,bhkd->bhqk", q, k) * (Dh ** -0.5)
    p = _softmax(scores, axis=-1)
    o = jnp.einsum("bhqk,bhkd->bhqd", p, v)
    return (lambda x, *d: x.transpose(*d))(o, 0, 2, 1, 3).reshape(B, Sq, Hq * Dh) @ wo
```

```python
import functools

import jax
import jax.numpy as jnp
import jax.experimental.pallas as pl
import jax.experimental.pallas.tpu as pltpu


def _kernel(x_ref, k_ref, v_ref, wq_ref, wo_ref, out_ref, q_scr, o_scr, *,
            sq, hkv, rep, dh, scale):
    b = pl.program_id(0)
    nb = pl.num_programs(0)

    @pl.when(b == 0)
    def _():
        q = jnp.dot(x_ref[...], wq_ref[...], preferred_element_type=jnp.float32)
        q_scr[...] = (q * scale).astype(q_scr.dtype)

    row0 = pl.multiple_of(b * sq, sq)
    for h in range(hkv):
        qh = jnp.concatenate(
            [q_scr[pl.ds(row0, sq), pl.ds((h * rep + r) * dh, dh)] for r in range(rep)],
            axis=0)
        k = k_ref[0, h]
        v = v_ref[0, h]
        s = jax.lax.dot_general(qh, k, (((1,), (1,)), ((), ())),
                                preferred_element_type=jnp.float32)
        m = jnp.max(s, axis=-1, keepdims=True)
        p = jnp.exp(s - m)
        l = jnp.sum(p, axis=-1, keepdims=True)
        o = jnp.dot(p.astype(v.dtype), v, preferred_element_type=jnp.float32)
        o = (o / l).astype(o_scr.dtype)
        for r in range(rep):
            o_scr[pl.ds(row0, sq), pl.ds((h * rep + r) * dh, dh)] = o[r * sq:(r + 1) * sq]

    @pl.when(b == nb - 1)
    def _():
        out_ref[...] = jnp.dot(o_scr[...], wo_ref[...],
                               preferred_element_type=jnp.float32).astype(out_ref.dtype)


@jax.jit
def pallas_standalone__gqa_block_cached__sampling_kernel(
    x: jax.Array,
    k_cache: jax.Array,
    v_cache: jax.Array,
    wq: jax.Array,
    wo: jax.Array,
):
    B, Sq, D = x.shape
    _, Hkv, Sk, Dh = k_cache.shape
    Hq = wq.shape[1] // Dh
    rep = Hq // Hkv
    x2 = x.reshape(B * Sq, D)

    kern = functools.partial(_kernel, sq=Sq, hkv=Hkv, rep=rep, dh=Dh, scale=Dh ** -0.5)
    out = pl.pallas_call(
        kern,
        grid=(B,),
        in_specs=[
            pl.BlockSpec((B * Sq, D), lambda b: (0, 0)),
            pl.BlockSpec((1, Hkv, Sk, Dh), lambda b: (b, 0, 0, 0)),
            pl.BlockSpec((1, Hkv, Sk, Dh), lambda b: (b, 0, 0, 0)),
            pl.BlockSpec((D, Hq * Dh), lambda b: (0, 0)),
            pl.BlockSpec((Hq * Dh, D), lambda b: (0, 0)),
        ],
        out_specs=pl.BlockSpec((B * Sq, D), lambda b: (0, 0)),
        out_shape=jax.ShapeDtypeStruct((B * Sq, D), x.dtype),
        scratch_shapes=[
            pltpu.VMEM((B * Sq, Hq * Dh), x.dtype),
            pltpu.VMEM((B * Sq, Hq * Dh), x.dtype),
        ],
        compiler_params=pltpu.CompilerParams(
            dimension_semantics=("arbitrary",),
            vmem_limit_bytes=100 * 1024 * 1024,
        ),
    )(x2, k_cache, v_cache, wq, wo)
    return out.reshape(B, Sq, D)
```

```python
import functools
import jax
import jax.numpy as jnp
import jax.experimental.pallas as pl
import jax.experimental.pallas.tpu as pltpu

NBUF = 4
GROUP = 8
UB = 4
NCH = 1024


def _kernel(x_hbm, k_hbm, v_hbm, wq_hbm, wo_hbm, out_hbm,
            x_buf, wq_buf, wo_buf, k_buf, v_buf, q_scr, o_scr, acc_scr, out_buf,
            sem_misc, sem_k, sem_v, sem_out, sem_tail, *, nb, sq, hkv, rep, dh, scale):
    hq_dh = wq_buf.shape[1]
    upg = GROUP // UB
    n_units = nb * hkv // UB
    grows = GROUP * sq
    last = n_units - 1

    def unit_coords(u):
        g = u // (hkv * upg)
        h = (u // upg) % hkv
        j = u % upg
        return g, h, j

    def k_copy(u, slot):
        g, h, j = unit_coords(u)
        b0 = g * GROUP + j * UB
        return pltpu.make_async_copy(k_hbm.at[pl.ds(b0, UB), h], k_buf.at[slot], sem_k.at[slot])

    def v_copy(u, slot):
        g, h, j = unit_coords(u)
        b0 = g * GROUP + j * UB
        return pltpu.make_async_copy(v_hbm.at[pl.ds(b0, UB), h], v_buf.at[slot], sem_v.at[slot])

    def k_copy_tail(i):
        g, h, j = unit_coords(last)
        b = g * GROUP + j * UB + i
        return pltpu.make_async_copy(k_hbm.at[b, h], k_buf.at[last % NBUF, i], sem_tail.at[2 * i])

    def v_copy_tail(i):
        g, h, j = unit_coords(last)
        b = g * GROUP + j * UB + i
        return pltpu.make_async_copy(v_hbm.at[b, h], v_buf.at[last % NBUF, i], sem_tail.at[2 * i + 1])

    def out_copy(g):
        r0 = pl.multiple_of(g * grows, grows)
        return pltpu.make_async_copy(out_buf.at[g % 2], out_hbm.at[pl.ds(r0, grows)],
                                     sem_out.at[g % 2])

    def attend(slot, i, row0, col0):
        qh = jnp.concatenate(
            [q_scr[pl.ds(row0, sq), pl.ds(col0 + r * dh, dh)] for r in range(rep)],
            axis=0)
        k = k_buf[slot, i]
        v = v_buf[slot, i]
        s = jax.lax.dot_general(qh, k, (((1,), (1,)), ((), ())),
                                preferred_element_type=jnp.float32)
        m = jnp.max(s, axis=-1, keepdims=True)
        p = jnp.exp(s - m)
        l = jnp.sum(p, axis=-1, keepdims=True)
        o = jnp.dot(p.astype(v.dtype), v, preferred_element_type=jnp.float32)
        o = (o / l).astype(o_scr.dtype)
        for r in range(rep):
            o_scr[pl.ds(row0, sq), pl.ds(col0 + r * dh, dh)] = o[r * sq:(r + 1) * sq]

    def out_proj_part(g, col0):
        g0 = pl.multiple_of(g * grows, grows)
        return jnp.dot(o_scr[pl.ds(g0, grows), pl.ds(col0, rep * dh)],
                       wo_buf[pl.ds(col0, rep * dh), :],
                       preferred_element_type=jnp.float32)

    x_cp = pltpu.make_async_copy(x_hbm, x_buf, sem_misc.at[0])
    wq_cp = pltpu.make_async_copy(wq_hbm, wq_buf, sem_misc.at[1])
    wo_cp = pltpu.make_async_copy(wo_hbm, wo_buf, sem_misc.at[2])

    x_cp.start()
    wq_cp.start()
    for s in range(NBUF):
        k_copy(s, s).start()
        v_copy(s, s).start()
    wo_cp.start()

    x_cp.wait()
    wq_cp.wait()
    for c in range(hq_dh // NCH):
        q = jnp.dot(x_buf[...], wq_buf[:, c * NCH:(c + 1) * NCH],
                    preferred_element_type=jnp.float32)
        q_scr[:, c * NCH:(c + 1) * NCH] = (q * scale).astype(q_scr.dtype)

    def body(u, carry):
        slot = u % NBUF
        g, h, j = unit_coords(u)
        col0 = pl.multiple_of(h * (rep * dh), rep * dh)
        k_copy(u, slot).wait()
        v_copy(u, slot).wait()
        for i in range(UB):
            row0 = pl.multiple_of((g * GROUP + j * UB + i) * sq, sq)
            attend(slot, i, row0, col0)

        @pl.when(u + NBUF < last)
        def _():
            k_copy(u + NBUF, slot).start()
            v_copy(u + NBUF, slot).start()

        @pl.when(u + NBUF == last)
        def _():
            for i in range(UB):
                k_copy_tail(i).start()
                v_copy_tail(i).start()

        @pl.when(j == upg - 1)
        def _():
            @pl.when(u == upg - 1)
            def _():
                wo_cp.wait()
            part = out_proj_part(g, col0)

            @pl.when(h == 0)
            def _():
                acc_scr[...] = part

            @pl.when(jnp.logical_and(h > 0, h < hkv - 1))
            def _():
                acc_scr[...] += part

            @pl.when(h == hkv - 1)
            def _():
                @pl.when(g >= 2)
                def _():
                    out_copy(g - 2).wait()
                out_buf[g % 2] = (acc_scr[...] + part).astype(out_buf.dtype)
                out_copy(g).start()
        return carry

    jax.lax.fori_loop(0, last, body, 0)

    g, h, j = unit_coords(last)
    col0 = h * (rep * dh)
    for i in range(UB):
        k_copy_tail(i).wait()
        v_copy_tail(i).wait()
        attend(last % NBUF, i, (g * GROUP + j * UB + i) * sq, col0)
    part = out_proj_part(g, col0)
    out_copy(g - 2).wait()
    out_buf[g % 2] = (acc_scr[...] + part).astype(out_buf.dtype)
    out_copy(g).start()
    out_copy(g - 1).wait()
    out_copy(g).wait()


@jax.jit
def pallas_standalone__gqa_block_cached__sampling_kernel(
    x: jax.Array,
    k_cache: jax.Array,
    v_cache: jax.Array,
    wq: jax.Array,
    wo: jax.Array,
):
    B, Sq, D = x.shape
    _, Hkv, Sk, Dh = k_cache.shape
    Hq = wq.shape[1] // Dh
    rep = Hq // Hkv
    x2 = x.reshape(B * Sq, D)

    kern = functools.partial(_kernel, nb=B, sq=Sq, hkv=Hkv, rep=rep, dh=Dh, scale=Dh ** -0.5)
    out = pl.pallas_call(
        kern,
        in_specs=[pl.BlockSpec(memory_space=pl.ANY)] * 5,
        out_specs=pl.BlockSpec(memory_space=pl.ANY),
        out_shape=jax.ShapeDtypeStruct((B * Sq, D), x.dtype),
        scratch_shapes=[
            pltpu.VMEM((B * Sq, D), x.dtype),
            pltpu.VMEM((D, Hq * Dh), wq.dtype),
            pltpu.VMEM((Hq * Dh, D), wo.dtype),
            pltpu.VMEM((NBUF, UB, Sk, Dh), k_cache.dtype),
            pltpu.VMEM((NBUF, UB, Sk, Dh), v_cache.dtype),
            pltpu.VMEM((B * Sq, Hq * Dh), x.dtype),
            pltpu.VMEM((B * Sq, Hq * Dh), x.dtype),
            pltpu.VMEM((GROUP * Sq, D), jnp.float32),
            pltpu.VMEM((2, GROUP * Sq, D), x.dtype),
            pltpu.SemaphoreType.DMA((3,)),
            pltpu.SemaphoreType.DMA((NBUF,)),
            pltpu.SemaphoreType.DMA((NBUF,)),
            pltpu.SemaphoreType.DMA((2,)),
            pltpu.SemaphoreType.DMA((2 * UB,)),
        ],
        compiler_params=pltpu.CompilerParams(
            vmem_limit_bytes=100 * 1024 * 1024,
        ),
    )(x2, k_cache, v_cache, wq, wo)
    return out.reshape(B, Sq, D)
```
